```python
import jax
import jax.numpy as jnp

def _softmax(x, axis=-1):
    return jax.nn.softmax(x, axis=axis)

def _gelu(x):
    return jax.nn.gelu(x, approximate=True)

def _silu(x):
    return jax.nn.silu(x)

def _sigmoid(x):
    return jax.nn.sigmoid(x)

def _layernorm(x, axis=-1, eps=1e-05):
    m = jnp.mean(x, axis=axis, keepdims=True)
    v = jnp.var(x, axis=axis, keepdims=True)
    return (x - m) / jnp.sqrt(v + eps)

def _scatter_add(tgt, idx, src, axis=0):
    return tgt.at[idx].add(src)

def _segment_sum(src, seg, n):
    return jax.ops.segment_sum(src, seg, n)

class _Rng:

    def __init__(self, key):
        self._k = key

    def _next(self):
        self._k, sub = jax.random.split(self._k)
        return sub

    def normal(self, shape):
        return jax.random.normal(self._next(), shape, dtype=jnp.bfloat16)

    def randint(self, lo, hi, shape):
        return jax.random.randint(self._next(), shape, lo, hi, dtype=jnp.int32)

    def uniform(self, shape, lo=0.0, hi=1.0):
        return jax.random.uniform(self._next(), shape, jnp.bfloat16, lo, hi)

    def permutation(self, n):
        return jax.random.permutation(self._next(), n)
kernel_name = 'sequential_preLN__ssm_conv_s4__mixer_gmlp__prompt'

def _fwd_setup_inputs():
    _rng = _Rng(jax.random.key(int.from_bytes(__import__("os").urandom(4), "little")))
    _w = lambda a: (lambda t: t.astype(jnp.bfloat16) if jnp.issubdtype(t.dtype, jnp.floating) else t)(jnp.asarray(a))

    def _A_setup():
        B, L, D, N = (1, 2048, 576, 128)
        A_re = -jnp.exp((lambda *s: _rng.normal(s) * 0.05)(D, N))
        A_im = jnp.pi * (lambda *s: _rng.normal(s) * 0.05)(D, N)
        B_re = (lambda *s: _rng.normal(s) * 0.05)(D, N)
        B_im = (lambda *s: _rng.normal(s) * 0.05)(D, N)
        C_re = (lambda *s: _rng.normal(s) * 0.05)(D, N)
        C_im = (lambda *s: _rng.normal(s) * 0.05)(D, N)
        log_dt = (lambda *s: _rng.normal(s) * 0.05)(D) * 0.5 - 4.0
        Dskip = (lambda *s: _rng.normal(s) * 0.05)(D)
        return {'u': _w((lambda *s: _rng.normal(s) * 0.05)(B, L, D)), 'A_re': _w(A_re), 'A_im': _w(A_im), 'B_re': _w(B_re), 'B_im': _w(B_im), 'C_re': _w(C_re), 'C_im': _w(C_im), 'log_dt': _w(log_dt), 'Dskip': _w(Dskip)}
    _A_in = _A_setup()

    def _B_setup():
        B, S, D, F = (1, 2048, 576, 4608)
        Fh = F // 2
        return {'x': _w((lambda *s: _rng.normal(s) * 0.05)(B, S, D)), 'w_in': _w((lambda *s: _rng.normal(s) * 0.05)(D, 2 * Fh)), 'w_sp': _w(0.01 * (lambda *s: _rng.normal(s) * 0.05)(S, S)), 'b_sp': _w(1.0 + 0.01 * (lambda *s: _rng.normal(s) * 0.05)(S)), 'w_out': _w((lambda *s: _rng.normal(s) * 0.05)(Fh, D))}
    _B_in = _B_setup()
    return {'A_u': _A_in['u'], 'A_A_re': _A_in['A_re'], 'A_A_im': _A_in['A_im'], 'A_B_re': _A_in['B_re'], 'A_B_im': _A_in['B_im'], 'A_C_re': _A_in['C_re'], 'A_C_im': _A_in['C_im'], 'A_log_dt': _A_in['log_dt'], 'A_Dskip': _A_in['Dskip'], 'B_x': _B_in['x'], 'B_w_in': _B_in['w_in'], 'B_w_sp': _B_in['w_sp'], 'B_b_sp': _B_in['b_sp'], 'B_w_out': _B_in['w_out']}

def _fwd_reference(A_u, A_A_re, A_A_im, A_B_re, A_B_im, A_C_re, A_C_im, A_log_dt, A_Dskip, B_x, B_w_in, B_w_sp, B_b_sp, B_w_out):

    def _A_ref(u, A_re, A_im, B_re, B_im, C_re, C_im, log_dt, Dskip):
        Bsz, L, D = u.shape
        dt = jnp.exp(log_dt)[:, None]
        A = A_re + 1j * A_im
        Bc = B_re + 1j * B_im
        Cc = C_re + 1j * C_im
        logdA = dt * A
        dB = dt * Bc
        l = (lambda x, dt: x.astype(dt))(jnp.arange(L), A_re.dtype)
        P = jnp.exp(logdA[:, :, None] * l[None, None, :])
        K = jnp.einsum('dn,dnl,dn->dl', Cc, P, dB).real
        L2 = 2 * L
        Kp = jnp.pad(K, ((0, 0), (0, L)))
        up = (lambda x, *d: x.transpose(*d))(u, 0, 2, 1)
        up = jnp.pad(up, ((0, 0), (0, 0), (0, L)))
        Kf = (lambda x, axes=(-2, -1): jnp.fft.rfft2(x.astype(jnp.float32), axes=axes))(Kp[:, None, :], axes=(-2, -1))
        Uf = (lambda x, axes=(-2, -1): jnp.fft.rfft2(x.astype(jnp.float32), axes=axes))(up[:, :, None, :], axes=(-2, -1))
        Yf = Uf * Kf[None, :, :, :]
        y = (lambda x, s, axes=(-2, -1): jnp.fft.irfft2(x, s=s, axes=axes).astype(jnp.bfloat16))(Yf, (1, L2), axes=(-2, -1))[:, :, 0, :L]
        y = (lambda x, *d: x.transpose(*d))(y, 0, 2, 1) + u * Dskip[None, None, :]
        return y

    def _B_ref(x, w_in, w_sp, b_sp, w_out):
        B, S, D = x.shape
        F = w_in.shape[-1]
        Fh = F // 2
        z = _gelu(jnp.einsum('bsd,df->bsf', x, w_in))
        z1 = z[..., :Fh].copy()
        z2 = _layernorm(z[..., Fh:], axis=-1)
        g = jnp.einsum('ts,bsf->btf', w_sp, z2) + b_sp[None, :, None]
        return jnp.einsum('bsf,fd->bsd', z1 * g, w_out)
    x = A_u
    h = x + _A_ref(_layernorm(x, axis=-1), A_A_re, A_A_im, A_B_re, A_B_im, A_C_re, A_C_im, A_log_dt, A_Dskip)
    h2 = h + _B_ref(_layernorm(h, axis=-1), B_w_in, B_w_sp, B_b_sp, B_w_out)
    return h2

def setup_inputs():
    _inp = _fwd_setup_inputs()
    _gk = jax.random.fold_in(jax.random.key(int.from_bytes(__import__("os").urandom(4), "little")), 2 ** 31 - 1)
    _shapes = [[1, 2048, 576]]
    _dtypes = ['bfloat16']
    _gks = jax.random.split(_gk, len(_shapes))
    _gs = [jax.random.normal(k, s, dtype=jnp.dtype(d)) * 0.05 for k, s, d in zip(_gks, _shapes, _dtypes)]
    _inp['grad_out'] = _gs[0]
    return _inp

def reference(A_u, A_A_re, A_A_im, A_B_re, A_B_im, A_C_re, A_C_im, A_log_dt, A_Dskip, B_w_in, B_w_sp, B_b_sp, B_w_out, B_x, grad_out):
    _const = dict(B_x=B_x)

    def _f(*_d):
        return _fwd_reference(**{'A_u': _d[0], 'A_A_re': _d[1], 'A_A_im': _d[2], 'A_B_re': _d[3], 'A_B_im': _d[4], 'A_C_re': _d[5], 'A_C_im': _d[6], 'A_log_dt': _d[7], 'A_Dskip': _d[8], 'B_w_in': _d[9], 'B_w_sp': _d[10], 'B_b_sp': _d[11], 'B_w_out': _d[12], **_const})
    _out, _vjp = jax.vjp(_f, A_u, A_A_re, A_A_im, A_B_re, A_B_im, A_C_re, A_C_im, A_log_dt, A_Dskip, B_w_in, B_w_sp, B_b_sp, B_w_out)
    _grads = _vjp(grad_out)
    _out0 = jnp.asarray(_out)
    return (_out0, *[jnp.asarray(_g) for _g in _grads])
```

```python
import numpy as np
import ml_dtypes
import jax
import jax.numpy as jnp
from jax import lax
import jax.experimental.pallas as pl
import jax.experimental.pallas.tpu as pltpu

f32 = jnp.float32
bf16 = jnp.bfloat16
u32 = jnp.uint32
L = 2048
D = 576
N = 128
F = 4608
FH = 2304
DP = 640
NG = 80
MP = 768
BT = 256
PR = 16
EPS = 1e-5
NN = (((1,), (0,)), ((), ()))
NT = (((1,), (1,)), ((), ()))
TN = (((0,), (0,)), ((), ()))
OCT_G = (32, 16, 16, 16)


def _pack_rows(a):
    u = np.ascontiguousarray(a.astype(ml_dtypes.bfloat16)).view(np.uint16).astype(np.uint32)
    return np.ascontiguousarray(u[..., 0::2, :] | (u[..., 1::2, :] << 16))


def _np_consts():
    npbf = ml_dtypes.bfloat16
    n1 = np.arange(16)
    F1h = np.zeros((32, 16))
    for j in range(32):
        F1h[j] = np.cos(2*np.pi*n1*j/32) if j <= 16 else -np.sin(2*np.pi*n1*(j-16)/32)
    F1k = np.kron(F1h, np.eye(8))
    n2 = np.arange(128)[:, None]
    k2 = np.arange(128)[None, :]

    def G(k1):
        ph = (n2 * (k1 + 32*k2)) % 4096
        return np.cos(2*np.pi*ph/4096), -np.sin(2*np.pi*ph/4096)
    Gall = np.zeros((16, 256, 256))
    g0r, g0i = G(0)
    g16r, g16i = G(16)
    Gall[0, :128] = np.concatenate([g0r, g0i], 1)
    Gall[0, 128:] = np.concatenate([g16r, g16i], 1)
    for s in range(1, 16):
        gr, gi = G(s)
        Gall[s, :128] = np.concatenate([gr, gi], 1)
        Gall[s, 128:] = np.concatenate([-gi, gr], 1)
    H = np.zeros((16, 16, 2))
    for a in range(16):
        H[a, 0, 0] = 1.0/4096
        H[a, 0, 1] = (-1.0)**a/4096
        for s in range(1, 16):
            th = 2*np.pi*a*s/32
            H[a, s, 0] = 2*np.cos(th)/4096
            H[a, s, 1] = -2*np.sin(th)/4096
    Hk = np.einsum('asp,de->adsep', H, np.eye(8)).reshape(128, 256)
    m = np.arange(MP)
    v = np.where(m < 256, m, np.where(m < 384, 256 + 2*(m-256), np.where(m < 512, 512 + 4*(m-384), 1024 + 8*(m-512))))
    lr = np.arange(L).astype(np.float32).astype(npbf).astype(np.float32).astype(np.int64)
    v2m = {int(v[i]): i for i in range(641)}
    idx = np.array([v2m[int(x)] for x in lr])
    pairs, blocks = [], []
    for a in range(16):
        for mt in range(6):
            blk = np.zeros((128, 128), np.float32)
            for j in range(128):
                mm = idx[a*128 + j] - mt*128
                if 0 <= mm < 128:
                    blk[mm, j] = 1.0
            if blk.any():
                pairs.append((a, mt))
                blocks.append(blk)
    return _pack_rows(F1k), _pack_rows(Gall), _pack_rows(Hk), _pack_rows(np.stack(blocks)), pairs


C_F1, C_G, C_H, C_SEL, SEL_PAIRS = _np_consts()


def _dot(a, b, dims=NN):
    return lax.dot_general(a, b, dims, preferred_element_type=f32)


def _cmul(a, b):
    return a[0]*b[0] - a[1]*b[1], a[0]*b[1] + a[1]*b[0]


def _csq(a):
    return a[0]*a[0] - a[1]*a[1], (a[0] + a[0])*a[1]


_GC = 0.7978845608028654
_GA = 0.044715


def _gelu(x):
    t = jnp.tanh(x * (_GC + (_GC*_GA) * (x*x)))
    return (0.5*x) * (1.0 + t)


def _gelu_and_grad(x):
    x2 = x*x
    t = jnp.tanh(x * (_GC + (_GC*_GA) * x2))
    hx = 0.5*x
    a = 0.5 + 0.5*t
    return x*a, a + hx*(1.0 - t*t)*(_GC + (3.0*_GC*_GA)*x2)


def _gelu_grad(x):
    return _gelu_and_grad(x)[1]


def _ds(start, size, mult):
    return pl.ds(pl.multiple_of(start, mult), size)


def _prow(r0, nr):
    if isinstance(r0, int):
        return slice(r0//2, (r0 + nr)//2)
    return pl.ds(pl.multiple_of(r0//2, 8), nr//2)


def pk(ref, r0, nr, cs=slice(None)):
    return pltpu.bitcast(ref[_prow(r0, nr), cs], bf16)


def pkst(ref, r0, cs, val):
    ref[_prow(r0, val.shape[0]), cs] = pltpu.bitcast(val.astype(bf16), u32)


def _bc(x):
    return pltpu.bitcast(x, bf16)


def _pu(x):
    return pltpu.bitcast(x.astype(bf16), u32)


def _colsum(x):
    r, c = x.shape
    return jnp.sum(x.reshape(r//8, 8, c), axis=0)


def _kernel(xT_h, Are_h, Aim_h, Bre_h, Bim_h, Cre_h, Cim_h, ldt_h, dsk_h,
            win_h, wsp_h, bsp_h, woutT_h, gT_h, F1_h, G_h, H_h, Sel_h,
            outT_h, dxT_h, dAre_h, dAim_h, dBre_h, dBim_h, dCre_h, dCim_h, dldt_h, ddsk_h,
            dwin_h, dwsp_h, dbsp_h, dwoutT_h,
            XG, F1, G, H, Sel, P, ldt_v, dsk_v, bsp_v, PT, dt_row, dskc, uT, hT, rows, Uf, Kf,
            ZY1, ZY2, YT, Z2nT, dGT, o1_v, o2_v, o3_v, sems):
    RX, RH, MH, R2, BS, DB, S1, S2, M1R, M2R = range(10)

    def cp(src, dst, i):
        return pltpu.make_async_copy(src, dst, sems.at[i])
    par_h = (Are_h, Aim_h, Bre_h, Bim_h, Cre_h, Cim_h)
    loads_small = [cp(par_h[i], P.at[i], i) for i in range(6)]
    loads_small += [cp(ldt_h, ldt_v, 6), cp(dsk_h, dsk_v, 7), cp(bsp_h, bsp_v, 8), cp(F1_h, F1, 9)]
    ld_H = cp(H_h, H, 10)
    ld_Sel = cp(Sel_h, Sel, 11)

    def ld_g(j):
        cs = _ds(j*BT, BT, BT)
        return pltpu.make_async_copy(gT_h.bitcast(u32).at[:, cs], XG.at[1, :, cs], sems.at[32 + j])
    ld_G = cp(G_h, G, 13)
    for c in loads_small:
        c.start()
    sub = lax.broadcasted_iota(jnp.int32, (8, 128), 0)
    b0 = (sub & 1) != 0
    b1 = (sub & 2) != 0
    b2 = (sub & 4) != 0

    def t1_vreg(row, q):
        e0 = (jnp.where(b0, row(0, q), 1.0), jnp.where(b0, row(1, q), 0.0))
        e1 = (jnp.where(b1, row(2, q), 1.0), jnp.where(b1, row(3, q), 0.0))
        e2 = (jnp.where(b2, row(4, q), 1.0), jnp.where(b2, row(5, q), 0.0))
        return _cmul(_cmul(e0, e1), e2)

    def _pe(a, b):
        return pltpu.bitcast(pltpu.pack_elementwise([a, b], packed_dtype=bf16), u32)

    def _ue(w):
        w = pltpu.bitcast(w, jnp.int32)
        return (pltpu.unpack_elementwise(w, index=0, packed_dtype=bf16, unpacked_dtype=f32),
                pltpu.unpack_elementwise(w, index=1, packed_dtype=bf16, unpacked_dtype=f32))

    def stage1_pair(src, dst, gp):
        base = pl.multiple_of(gp*16, 16)
        outs = []
        for hh in range(2):
            r = src[:, pl.ds(base + hh, 8, stride=2), :].reshape(128, 128).astype(bf16)
            outs.append(_dot(_bc(F1[...]), r))
        dst[:, _prow(gp*16, 16), :] = _pe(outs[0], outs[1]).reshape(32, 8, 128)

    def store_B(dst, s, bre, bim):
        dst[:, _prow(s*16, 16), :] = _pe(bre, bim).reshape(72, 8, 128)

    def spec(A, s):
        g = _bc(G[s])
        return _dot(_bc(A[s]), g[0:128]) + _dot(_bc(A[16+s]), g[128:256])

    def h2d(i):
        return jnp.concatenate([hT[2*i], hT[2*i + 1]], axis=1)

    def powers(t):
        dtv = dt_row[...]
        ar = PT[0, t]*dtv
        ai = PT[1, t]*dtv
        mag = jnp.exp(ar)
        Es = [(mag*jnp.cos(ai), mag*jnp.sin(ai))]
        for p in range(10):
            Es.append(_csq(Es[-1]))
        return Es, dtv

    def w1_scope(win, woutT):
        ld_win = cp(win_h.bitcast(u32), win, 14)
        ld_wout = cp(woutT_h.bitcast(u32), woutT, 16)

        def fwd_scope(xT, tabs, Kd, KdT, KT, A_u, A_k, B_s, st1, st2):
            ld_x = cp(xT_h.bitcast(u32), xT, 17)
            ld_x.start()
            ld_g(0).start()
            ld_wout.start()
            for c in loads_small:
                c.wait()
            for i in range(6):
                pf = P[i].astype(f32)
                aug = jnp.concatenate([pf, pltpu.roll(pf[512:576], 124, 1)], axis=0)
                PT[i] = aug.T.reshape(16, 8, DP)
            dt_row[...] = jnp.zeros(dt_row.shape, f32)
            dt = jnp.exp(ldt_v[...].astype(f32).reshape(1, D)).astype(bf16).astype(f32)
            dt_row[:, 0:D] = dt
            d4 = jnp.broadcast_to(dt_row[:, 512:640], (8, 128))
            dt_row[:, 512:640] = (d4 + pltpu.roll(d4, 64, 1))[0:1]
            dskc[...] = jnp.broadcast_to(dsk_v[...].astype(f32).reshape(1, D), (128, D)).T

            def tab_body(t, _):
                Es, dtv = powers(t)
                w = _cmul((PT[4, t], PT[5, t]), (PT[2, t]*dtv, PT[3, t]*dtv))
                for p in range(3):
                    tabs[2*p, t] = Es[p][0]
                    tabs[2*p+1, t] = Es[p][1]
                for o in range(4):
                    R = Es[3+o]
                    tabs[6+2*o, t] = R[0] + R[0]
                    tabs[7+2*o, t] = R[0]*R[0] + R[1]*R[1]
                    Bo = w if o == 0 else _cmul(w, Es[7+o])
                    BR = _cmul(Bo, R)
                    tabs[14+4*o, t] = Bo[0]
                    tabs[15+4*o, t] = Bo[1]
                    tabs[16+4*o, t] = BR[0]
                    tabs[17+4*o, t] = BR[1]
                E11 = _csq(Es[10])
                tabs[30, t] = w[0]*E11[0] - w[1]*E11[1]
                return 0
            with jax.named_scope('tab'):
                lax.fori_loop(0, 16, tab_body, 0)
            Kd[...] = jnp.zeros(Kd.shape, f32)
            k640 = tabs[30, 0]
            for t in range(1, 16):
                k640 = k640 + tabs[30, t]
            sub6 = lax.broadcasted_iota(jnp.int32, (8, DP), 0)
            lane6 = lax.broadcasted_iota(jnp.int32, (8, DP), 1)
            k640 = jnp.where((lane6 < 512) | (sub6 < 4), k640, 0.0)
            Kd[640:648, :] = jnp.where(sub6 == 0, jnp.sum(k640, axis=0, keepdims=True), 0.0)
            ld_x.wait()

            def ln_body(c, _):
                cs = _ds(c*128, 128, 128)
                xt = pk(xT, 0, D, cs).astype(f32)
                m = jnp.sum(xt, axis=0, keepdims=True) * (1.0/D)
                xc = xt - m
                v = jnp.sum(xc*xc, axis=0, keepdims=True) * (1.0/D)
                r = lax.rsqrt(v + EPS)
                uT[c] = xc*r
                rows[RX:RX+1, cs] = r
                return 0
            with jax.named_scope('ln1'):
                lax.fori_loop(0, 16, ln_body, 0, unroll=2)

            def kgen_unit(t, tile):
                ls = slice(tile*128, tile*128 + 128)

                def row(i, q):
                    return jnp.broadcast_to(tabs[i, t, q:q+1, ls], (8, 128))
                for q0 in range(0, 8 if tile < 4 else 4, 2):
                    Ts = [t1_vreg(row, q) for q in (q0, q0+1)]
                    g0 = 0
                    for o in range(4):
                        qa, qb, c1, c2 = [], [], [], []
                        for k, q in enumerate((q0, q0+1)):
                            T = Ts[k]
                            qa.append(row(14+4*o, q)*T[0] - row(15+4*o, q)*T[1])
                            qb.append(row(16+4*o, q)*T[0] - row(17+4*o, q)*T[1])
                            c1.append(row(6+2*o, q))
                            c2.append(row(7+2*o, q))
                            if o < 3:
                                Ts[k] = _csq(T)
                        for g in range(OCT_G[o]):
                            rs = slice((g0+g)*8, (g0+g)*8 + 8)
                            Kd[rs, ls] = Kd[rs, ls] + (qa[0] + qa[1])
                            if g + 2 < OCT_G[o]:
                                for k in range(2):
                                    nxt = c1[k]*qb[k] - c2[k]*qa[k]
                                    qa[k] = qb[k]
                                    qb[k] = nxt
                            else:
                                for k in range(2):
                                    qa[k] = qb[k]
                        g0 += OCT_G[o]

            for j in range(1, 8):
                ld_g(j).start()
            ld_wout.wait()
            ld_G.start()
            ld_Sel.start()
            ld_H.start()

            def front(i, extra):
                cs = _ds(i*BT, BT, BT)
                ld_g(i).wait()
                gb = pk(XG.at[1], 0, D, cs)
                k = 0
                for tt in range(2):
                    for tile in range(5):
                        kgen_unit(2*i + tt, tile)
                        if k < 9:
                            pkst(dGT, k*256, cs, _dot(pk(woutT, 0, D, slice(k*256, (k+1)*256)), gb, TN))
                            extra(i, k)
                            k += 1

            def front1(i, _):
                front(i, lambda i, k: stage1_pair(uT, A_u, i*9 + k))
                return 0

            def ex2(i, k):
                if k % 2 == 1:
                    s = jnp.minimum(1 + (i - 4)*4 + k//2, 15)
                    U = spec(A_u, s)
                    Uf[s] = _pe(U[:, :128], U[:, 128:])

            def front2(i, _):
                front(i, ex2)
                return 0
            with jax.named_scope('front1'):
                lax.fori_loop(0, 4, front1, 0)
            ld_G.wait()
            ld_win.start()
            with jax.named_scope('front2'):
                lax.fori_loop(4, 8, front2, 0)

            k4 = Kd[:, 512:640]
            Kd[:, 512:640] = k4 + pltpu.roll(k4, 64, 1)
            KdT[...] = _pu(Kd[...].T)
            ld_Sel.wait()
            ld_H.wait()
            acc = {}
            for i, (a, mt) in enumerate(SEL_PAIRS):
                r = _dot(pk(KdT, 0, D, slice(mt*128, (mt+1)*128)), _bc(Sel[i]))
                acc[a] = r if a not in acc else acc[a] + r
            for a in range(16):
                KT[a] = acc[a]

            def st1k(it, _):
                for j in range(18):
                    stage1_pair(KT, A_k, it*18 + j)
                return 0
            with jax.named_scope('st1k'):
                lax.fori_loop(0, 2, st1k, 0)

            def cm(a, b):
                ar, ai, br, bi = a[:, :128], a[:, 128:], b[:, :128], b[:, 128:]
                return jnp.concatenate([ar*br - ai*bi, ar*bi + ai*br], axis=1).astype(bf16)
            g0 = _bc(G[0])
            U0 = _dot(_bc(A_u[0]), g0[0:128])
            U16 = _dot(_bc(A_u[16]), g0[128:256])
            K0 = _dot(_bc(A_k[0]), g0[0:128])
            K16 = _dot(_bc(A_k[16]), g0[128:256])
            for j, v in ((0, U0), (16, U16)):
                Uf[j] = _pe(v[:, :128], v[:, 128:])
            for j, v in ((0, K0), (16, K16)):
                Kf[j] = _pe(v[:, :128], v[:, 128:])
            store_B(B_s, 0, _dot(cm(U0, K0), g0[0:128], NT), _dot(cm(U16, K16), g0[128:256], NT))

            def k1_body(s, _):
                K = spec(A_k, s)
                Kf[s] = _pe(K[:, :128], K[:, 128:])
                B = _dot(cm(jnp.concatenate(_ue(Uf[s]), axis=1), K), _bc(G[s]), NT)
                store_B(B_s, s, B[:, :128], B[:, 128:])
                return 0
            with jax.named_scope('k1f'):
                lax.fori_loop(1, 16, k1_body, 0, unroll=3)

            st1[...] = jnp.zeros(st1.shape, f32)
            st2[...] = jnp.zeros(st2.shape, f32)

            def inv1_body(it, _):
                s1 = st1[...]
                s2 = st2[...]
                for j in range(9):
                    gp = it*9 + j
                    rs = _ds(gp*16, 16, 16)
                    ys = [_dot(_bc(H[...]), _bc(B_s[gp*2 + hh])).reshape(16, 8, 128) for hh in range(2)]
                    y = jnp.concatenate(ys, axis=1)
                    xw = pk(xT, gp*16, 16).astype(f32)
                    x3 = jnp.stack([xw[:, a*128:(a+1)*128] for a in range(16)], axis=0)
                    h = x3 + uT[:, rs, :]*dskc[rs, :][None] + y
                    hT[:, rs, :] = h
                    s1 = s1 + (h[:, 0:8] + h[:, 8:16])
                    h2 = h*h
                    s2 = s2 + (h2[:, 0:8] + h2[:, 8:16])
                st1[...] = s1
                st2[...] = s2
                return 0
            with jax.named_scope('inv1f'):
                lax.fori_loop(0, 4, inv1_body, 0)
            for c in range(16):
                cs = slice(c*128, (c+1)*128)
                rows[S1:S1+1, cs] = jnp.sum(st1[c], axis=0, keepdims=True)
                rows[S2:S2+1, cs] = jnp.sum(st2[c], axis=0, keepdims=True)
            mh = rows[S1:S1+1, :]*(1.0/D)
            rows[MH:MH+1, :] = mh
            rows[RH:RH+1, :] = lax.rsqrt(rows[S2:S2+1, :]*(1.0/D) - mh*mh + EPS)

        pl.run_scoped(fwd_scope,
                      pltpu.VMEM((D//2, L), u32), pltpu.VMEM((31, 16, 8, DP), f32), pltpu.VMEM((MP, DP), f32),
                      pltpu.VMEM((DP//2, MP), u32), pltpu.VMEM((16, D, 128), f32),
                      pltpu.VMEM((32, D//2, 128), u32), pltpu.VMEM((32, D//2, 128), u32),
                      pltpu.VMEM((72, 128, 128), u32), pltpu.VMEM((16, 8, 128), f32), pltpu.VMEM((16, 8, 128), f32))

        def b_scope(wsp, DZ, dXs, out_v, st, db8, WS, sl1, sl2):
            ld_wsp = cp(wsp_h.bitcast(u32), wsp, 15)
            ld_wsp.start()
            ld_win.wait()
            st[...] = jnp.ones(st.shape, f32)
            Z2nT[:, 0:BT] = jnp.zeros((FH//2, BT), u32)

            def p1_body(i, _):
                cs = _ds(i*BT, BT, BT)
                cp_ = _ds(jnp.maximum(i - 1, 0)*BT, BT, BT)
                mprev = st[0:1, :]
                rprev = st[1:2, :]
                xb = ((h2d(i) - rows[MH:MH+1, cs]) * rows[RH:RH+1, cs]).astype(bf16)
                pkst(XG.at[0], 0, cs, xb)
                s1 = jnp.zeros((8, BT), f32)
                s2 = jnp.zeros((8, BT), f32)
                for k in range(9):
                    for j in range(16):
                        r0 = k*256 + j*16
                        pkst(Z2nT, r0, cp_, (pk(Z2nT, r0, 16, cp_).astype(f32) - mprev) * rprev)
                    z = _dot(pk(win, 0, D, slice(FH + k*256, FH + (k+1)*256)), xb, TN)
                    pkst(ZY2, k*256, cs, z)
                    g = _gelu(z)
                    z1 = _dot(pk(win, 0, D, slice(k*256, (k+1)*256)), xb, TN)
                    pkst(ZY1, k*256, cs, z1)
                    s1 = s1 + _colsum(g)
                    s2 = s2 + _colsum(g*g)
                    pkst(Z2nT, k*256, cs, g)
                m = jnp.sum(s1, axis=0, keepdims=True) * (1.0/FH)
                vv = jnp.sum(s2, axis=0, keepdims=True) * (1.0/FH) - m*m
                r = lax.rsqrt(vv + EPS)
                rows[R2:R2+1, cs] = r
                st[0:1, :] = m
                st[1:2, :] = r
                return 0
            with jax.named_scope('p1'):
                lax.fori_loop(0, 8, p1_body, 0)
            lastc = slice(7*BT, 8*BT)
            for k in range(9):
                pkst(Z2nT, k*256, lastc, (pk(Z2nT, k*256, 256, lastc).astype(f32) - st[0:1, :]) * st[1:2, :])
            ld_wsp.wait()
            rows[BS:BS+1, :] = bsp_v[...].astype(f32).reshape(1, L)
            db8[...] = jnp.zeros(db8.shape, f32)

            h1 = slice(0, L//2)
            h2 = slice(L//2, L)

            def ws_body(i, _):
                r = i*128
                w11 = pk(wsp, r, 128, h1).astype(f32)
                w12 = pk(wsp, r, 128, h2).astype(f32)
                w21 = pk(wsp, L//2 + r, 128, h1).astype(f32)
                w22 = pk(wsp, L//2 + r, 128, h2).astype(f32)
                for j, v in enumerate((w11 + w22, w21 - w22, w12 - w11, w11 + w21, w12 + w22)):
                    pkst(WS.at[j], r, slice(None), v)
                return 0
            with jax.named_scope('wsum'):
                lax.fori_loop(0, 8, ws_body, 0)

            def p2_body(i, _):
                r1 = i*128
                r2 = FH//2 + i*128

                def epi(Gm, r0, cs):
                    z1, gp = _gelu_and_grad(pk(ZY1, r0, 128, cs).astype(f32))
                    pkst(YT, r0, cs, z1*Gm)
                    dy = pk(dGT, r0, 128, cs).astype(f32)
                    dG = dy*z1
                    pkst(dGT, r0, cs, dG)
                    db8[:, cs] = db8[:, cs] + _colsum(dG)
                    pkst(ZY1, r0, cs, dy*Gm*gp)
                b11 = pk(Z2nT, r1, 128, h1)
                b12 = pk(Z2nT, r1, 128, h2)
                b21 = pk(Z2nT, r2, 128, h1)
                b22 = pk(Z2nT, r2, 128, h2)
                a11, a12, a21, a22 = [x.astype(f32) for x in (b11, b12, b21, b22)]
                W11 = pk(wsp, 0, L//2, h1)
                W22 = pk(wsp, L//2, L//2, h2)
                ws = [_bc(WS[j]) for j in range(5)]
                br = rows[BS:BS+1, :]
                M2 = _dot((a21 + a22).astype(bf16), W11, NT)
                M4 = _dot(b22, ws[2], NT)
                epi(M2 + M4 + br[:, h1], r2, h1)
                M3 = _dot(b11, ws[1], NT)
                M5 = _dot((a11 + a12).astype(bf16), W22, NT)
                epi(M3 + M5 + br[:, h2], r1, h2)
                M1 = _dot((a11 + a22).astype(bf16), ws[0], NT)
                M7 = _dot((a12 - a22).astype(bf16), ws[4], NT)
                epi((M4 - M5) + (M1 + M7) + br[:, h1], r1, h1)
                M6 = _dot((a21 - a11).astype(bf16), ws[3], NT)
                epi((M3 - M2) + (M1 + M6) + br[:, h2], r2, h2)
                return 0
            with jax.named_scope('p2'):
                lax.fori_loop(0, 9, p2_body, 0)
            o3_v[...] = jnp.sum(db8[...], axis=0, keepdims=True).reshape(L).astype(bf16)
            st_db = cp(o3_v, dbsp_h, 18)
            st_db.start()

            sl1[...] = jnp.zeros(sl1.shape, f32)
            sl2[...] = jnp.zeros(sl2.shape, f32)

            def p4_body(i, _):
                r1 = i*128
                r2 = FH//2 + i*128

                def epi(C, r0, cs):
                    xh = pk(Z2nT, r0, 128, cs).astype(f32)
                    sl1[:, cs] = sl1[:, cs] + _colsum(C)
                    sl2[:, cs] = sl2[:, cs] + _colsum(C*xh)
                    pkst(DZ, r0, cs, C)
                b11 = pk(dGT, r1, 128, h1)
                b12 = pk(dGT, r1, 128, h2)
                b21 = pk(dGT, r2, 128, h1)
                b22 = pk(dGT, r2, 128, h2)
                a11, a12, a21, a22 = [x.astype(f32) for x in (b11, b12, b21, b22)]
                W11 = pk(wsp, 0, L//2, h1)
                W22 = pk(wsp, L//2, L//2, h2)
                ws = [_bc(WS[j]) for j in range(5)]
                M2 = _dot(b11, ws[4])
                M4 = _dot((a12 - a11).astype(bf16), W22)
                epi(M2 + M4, r1, h2)
                M3 = _dot((a21 - a22).astype(bf16), W11)
                M5 = _dot(b22, ws[3])
                epi(M3 + M5, r2, h1)
                M1 = _dot((a11 + a22).astype(bf16), ws[0])
                M7 = _dot((a12 + a22).astype(bf16), ws[1])
                epi((M4 - M5) + (M1 + M7), r1, h1)
                M6 = _dot((a11 + a21).astype(bf16), ws[2])
                epi((M3 - M2) + (M1 + M6), r2, h2)
                return 0
            with jax.named_scope('p4'):
                lax.fori_loop(0, 9, p4_body, 0)
            rows[M1R:M1R+1, :] = jnp.sum(sl1[...], axis=0, keepdims=True) * (1.0/FH)
            rows[M2R:M2R+1, :] = jnp.sum(sl2[...], axis=0, keepdims=True) * (1.0/FH)

            def piece(r0, nr, cs):
                xh = pk(Z2nT, r0, nr, cs).astype(f32)
                dz = rows[R2:R2+1, cs] * (pk(DZ, r0, nr, cs).astype(f32) - rows[M1R:M1R+1, cs] - xh*rows[M2R:M2R+1, cs])
                gp = _gelu_grad(pk(ZY2, r0, nr, cs).astype(f32))
                pkst(ZY2, r0, cs, dz*gp)

            def pa_body(i, _):
                cs = _ds(i*BT, BT, BT)
                for c in range(8):
                    for j in range(288 // PR):
                        piece(i*288 + j*PR, PR, slice(c*BT, (c+1)*BT))
                O = _dot(_bc(woutT[...]), pk(YT, 0, FH, cs))
                pkst(out_v, 0, cs, h2d(i) + O)
                dXa = _dot(pk(win, 0, D, slice(0, FH)), pk(ZY1, 0, FH, cs))
                dXs[2*i] = dXa[:, 0:128]
                dXs[2*i + 1] = dXa[:, 128:256]
                return 0
            with jax.named_scope('pa'):
                lax.fori_loop(0, 8, pa_body, 0)
            st_out = cp(out_v, outT_h.bitcast(u32), 19)
            st_out.start()

            def lnh_tile(c, cd):
                cs_ = _ds(cd*128, 128, 128)
                dX = dXs[c]
                xh2 = pk(XG.at[0], 0, D, cs_).astype(f32)
                n1 = jnp.sum(dX, axis=0, keepdims=True) * (1.0/D)
                n2 = jnp.sum(dX*xh2, axis=0, keepdims=True) * (1.0/D)
                r = rows[RH:RH+1, cs_]
                for j in range(D // 16):
                    rs = slice(j*16, (j+1)*16)
                    v = pk(XG.at[1], j*16, 16, cs_).astype(f32) + r * (dXs[c, rs, :] - n1 - pk(XG.at[0], j*16, 16, cs_).astype(f32)*n2)
                    dXs[c, rs, :] = v
                    hT[cd, rs, :] = v

            def lnh(ib, src):
                lnh_tile(src, 2*ib)
                lnh_tile(src + 1, 2*ib + 1)
            dXs[16:18] = jnp.zeros((2, D, 128), f32)

            def pb_body(i, _):
                cs = _ds(i*BT, BT, BT)
                lnh(jnp.maximum(i - 1, 0), jnp.where(i == 0, 16, 2*i - 2))
                dXb = _dot(pk(win, 0, D, slice(FH, F)), pk(ZY2, 0, FH, cs))
                dXs[2*i] = dXs[2*i] + dXb[:, 0:128]
                dXs[2*i + 1] = dXs[2*i + 1] + dXb[:, 128:256]
                return 0
            with jax.named_scope('pb'):
                lax.fori_loop(0, 8, pb_body, 0)
            lnh(7, 14)
            st_db.wait()
            st_out.wait()
        pl.run_scoped(b_scope, pltpu.VMEM((L//2, L), u32), pltpu.VMEM((FH//2, L), u32), pltpu.VMEM((18, D, 128), f32),
                      pltpu.VMEM((D//2, L), u32), pltpu.VMEM((8, BT), f32), pltpu.VMEM((8, L), f32),
                      pltpu.VMEM((5, L//4, L//2), u32), pltpu.VMEM((8, L), f32), pltpu.VMEM((8, L), f32))

    pl.run_scoped(w1_scope, pltpu.VMEM((D//2, F), u32), pltpu.VMEM((D//2, FH), u32))

    def bwd_scope(tabs, cc, GG, dxv, dKdT, duT, c640, PG):
        def s1_scope(A_d, B_du, B_dk, dKT, acc_ds):
            def st1d(it, _):
                for j in range(18):
                    stage1_pair(hT, A_d, it*18 + j)
                return 0
            with jax.named_scope('st1d'):
                lax.fori_loop(0, 2, st1d, 0)

            def cmc(a, b):
                ar, ai = a[:, :128], a[:, 128:]
                br, bi = _ue(b)
                return jnp.concatenate([ar*br + ai*bi, ai*br - ar*bi], axis=1).astype(bf16)

            def tab_b(t):
                Es, dtv = powers(t)
                for p in range(3):
                    tabs[2*p, t] = Es[p][0]
                    tabs[2*p+1, t] = Es[p][1]
                for o in range(4):
                    R = Es[3+o]
                    tabs[6+2*o, t] = R[0] + R[0]
                    tabs[7+2*o, t] = R[0]*R[0] + R[1]*R[1]
                    tabs[14+2*o, t] = R[0]
                    tabs[15+2*o, t] = R[1]
                    if o > 0:
                        tabs[22+2*(o-1), t] = Es[7+o][0]
                        tabs[23+2*(o-1), t] = Es[7+o][1]
                E11 = _csq(Es[10])
                tabs[28, t] = E11[0]
                tabs[29, t] = E11[1]
            g0 = _bc(G[0])
            tab_b(0)
            D0 = _dot(_bc(A_d[0]), g0[0:128])
            D16 = _dot(_bc(A_d[16]), g0[128:256])
            store_B(B_du, 0, _dot(cmc(D0, Kf[0]), g0[0:128], NT), _dot(cmc(D16, Kf[16]), g0[128:256], NT))
            store_B(B_dk, 0, _dot(cmc(D0, Uf[0]), g0[0:128], NT), _dot(cmc(D16, Uf[16]), g0[128:256], NT))

            def k1_body(s, _):
                tab_b(s)
                g = _bc(G[s])
                Dy = spec(A_d, s)
                B1 = _dot(cmc(Dy, Kf[s]), g, NT)
                store_B(B_du, s, B1[:, :128], B1[:, 128:])
                B2 = _dot(cmc(Dy, Uf[s]), g, NT)
                store_B(B_dk, s, B2[:, :128], B2[:, 128:])
                return 0
            with jax.named_scope('k1b'):
                lax.fori_loop(1, 16, k1_body, 0)

            def inv1_body(it, _):
                for j in range(6):
                    gp = it*6 + j
                    os_ = [_dot(_bc(H[...]), jnp.concatenate([_bc(B_du[gp*2 + hh]), _bc(B_dk[gp*2 + hh])], axis=1))
                           for hh in range(2)]
                    rs = _ds(gp*16, 16, 16)
                    du = jnp.concatenate([o[:, 0:128].reshape(16, 8, 128) for o in os_], axis=1)
                    dk = jnp.concatenate([o[:, 128:256].reshape(16, 8, 128) for o in os_], axis=1)
                    for a in range(16):
                        dKT[a, _prow(gp*16, 16), :] = _pu(dk[a])
                    dy = hT[:, rs, :]
                    duT[:, rs, :] = du + dy*dskc[rs, :][None]
                    acc_ds[rs, :] = jnp.sum(dy*uT[:, rs, :], axis=0)
                return 0
            with jax.named_scope('inv1b'):
                lax.fori_loop(0, 6, inv1_body, 0)

            acc = {}
            for i, (a, mt) in enumerate(SEL_PAIRS):
                r = _dot(_bc(dKT[a]), _bc(Sel[i]), NT)
                acc[mt] = r if mt not in acc else acc[mt] + r
            for mt in range(6):
                dKdT[0:D, mt*128:(mt+1)*128] = acc[mt]
                dKdT[D:DP, mt*128:(mt+1)*128] = acc[mt][512:576]
            cT = dKdT[...].T
            mi = lax.broadcasted_iota(jnp.int32, (NG*8, 128), 0)
            vi = jnp.where(mi < 256, mi, jnp.where(mi < 384, 2*mi - 256, jnp.where(mi < 512, 4*mi - 1024, 8*mi - 3072)))
            vf = vi.astype(f32)
            c0 = cT[0:NG*8]
            cc[0] = c0
            cc[1] = c0 * jnp.concatenate([vf]*5, axis=1)
            c640[...] = cT[640:648]

            acc_ds[D:DP, :] = jnp.zeros((DP - D, 128), f32)
            asum = jnp.sum(acc_ds[...].T, axis=0, keepdims=True)
            o1_v[...] = asum[:, 0:D].reshape(D).astype(bf16)
            cp(o1_v, ddsk_h, 20).start()

        pl.run_scoped(s1_scope, pltpu.VMEM((32, D//2, 128), u32), pltpu.VMEM((72, 128, 128), u32), pltpu.VMEM((72, 128, 128), u32),
                      pltpu.VMEM((16, D//2, 128), u32), pltpu.VMEM((DP, 128), f32))

        GG[...] = jnp.zeros(GG.shape, f32)

        def goertzel(t, tile):
            ls = slice(tile*128, tile*128 + 128)

            def row(i, q):
                return jnp.broadcast_to(tabs[i, t, q:q+1, ls], (8, 128))
            for q in range(8 if tile < 4 else 4):
                T = t1_vreg(row, q)
                tot = [None, None]
                g0 = 0
                for o in range(4):
                    c1 = row(6+2*o, q)
                    c2 = row(7+2*o, q)
                    bb1 = [None, None]
                    bb2 = [None, None]
                    for g in range(OCT_G[o]-1, -1, -1):
                        rs = slice((g0+g)*8, (g0+g)*8 + 8)
                        for ch in range(2):
                            cv = cc[ch, rs, ls]
                            if bb1[ch] is None:
                                nb = cv
                            elif bb2[ch] is None:
                                nb = cv + c1*bb1[ch]
                            else:
                                nb = cv + c1*bb1[ch] - c2*bb2[ch]
                            bb2[ch] = bb1[ch]
                            bb1[ch] = nb
                    Rr = row(14+2*o, q)
                    Ri = row(15+2*o, q)
                    for ch in range(2):
                        S = _cmul((bb1[ch] - Rr*bb2[ch], Ri*bb2[ch]), T)
                        if o > 0:
                            S = _cmul(S, (row(22+2*(o-1), q), row(23+2*(o-1), q)))
                            tot[ch] = (tot[ch][0] + S[0], tot[ch][1] + S[1])
                        else:
                            tot[ch] = S
                    if o < 3:
                        T = _csq(T)
                    g0 += OCT_G[o]
                for ch in range(2):
                    for part in range(2):
                        GG[2*ch+part, t, q:q+1, ls] = jnp.sum(tot[ch][part], axis=0, keepdims=True)

        def dx_tile(c):
            du = duT[c]
            u = uT[c]
            cs = _ds(c*128, 128, 128)
            m1 = jnp.sum(du, axis=0, keepdims=True) * (1.0/D)
            m2 = jnp.sum(du*u, axis=0, keepdims=True) * (1.0/D)
            pkst(dxv, 0, cs, hT[c] + rows[RX:RX+1, cs] * (du - m1 - u*m2))

        def pgrad(t):
            dtv = dt_row[...]
            Ar, Ai, Br, Bi, Cr, Ci = [PT[i, t] for i in range(6)]
            Dr, Di = Br*dtv, Bi*dtv
            wr, wi = _cmul((Cr, Ci), (Dr, Di))
            cl = c640[0:1, :]
            er, ei = cl*tabs[28, t], cl*tabs[29, t]
            gwr, gwi = GG[0, t] + er, -(GG[1, t] + ei)
            G1r, G1i = GG[2, t] + 2048.0*er, GG[3, t] + 2048.0*ei
            gar = wr*G1r - wi*G1i
            gai = -(wr*G1i + wi*G1r)
            gDr = gwr*Cr + gwi*Ci
            gDi = gwi*Cr - gwr*Ci
            vals = (gar*dtv, gai*dtv, gDr*dtv, gDi*dtv, gwr*Dr + gwi*Di, gwi*Dr - gwr*Di,
                    gDr*Br + gDi*Bi + gar*Ar + gai*Ai)
            for i, v in enumerate(vals):
                PG[i, t] = v

        def final_copies():
            pg_h = (dAre_h, dAim_h, dBre_h, dBim_h, dCre_h, dCim_h)
            return [cp(P.at[i], pg_h[i], i) for i in range(6)] + [cp(o2_v, dldt_h, 6)]

        def finish():
            dtv = dt_row[...]
            gacc = PG[6, 0]
            for t in range(1, 16):
                gacc = gacc + PG[6, t]
            lane = lax.broadcasted_iota(jnp.int32, (64, 128), 1)
            lowq = (lane & 4) == 0
            for i in range(6):
                T = PG[i].reshape(128, DP).T
                P[i, 0:512, :] = T[0:512].astype(bf16)
                P[i, 512:576, :] = jnp.where(lowq, T[512:576], pltpu.roll(T[576:640], 4, 1)).astype(bf16)
            g4 = gacc[:, 512:640]
            gfull = jnp.concatenate([gacc[:, 0:512], g4 + pltpu.roll(g4, 64, 1)], axis=1)
            o2_v[...] = (jnp.sum(gfull, axis=0, keepdims=True) * dtv)[:, 0:D].reshape(D).astype(bf16)
            for c in final_copies():
                c.start()

        def s2_scope(stg, stg2):
            def st_a(slot, rs):
                return pltpu.make_async_copy(stg.at[slot], dwsp_h.bitcast(u32).at[rs, :], sems.at[22 + slot])

            def wsp_body(i, _):
                slot = i % 2
                rs = _ds(i*128, 128, 128)

                @pl.when(i >= 2)
                def _():
                    st_a(slot, rs).wait()
                for tile in range(5):
                    goertzel(i, tile)
                goertzel(8 + i, 0)
                pgrad(i)
                stg[slot] = _pu(_dot(pk(dGT, 0, FH, _ds(i*256, 256, 256)), _bc(Z2nT[...]), TN))
                st_a(slot, rs).start()
                return 0
            with jax.named_scope('wsp'):
                lax.fori_loop(0, 8, wsp_body, 0)

            def st_b(slot, dst, j):
                return pltpu.make_async_copy(stg2.at[slot], dst.bitcast(u32).at[:, _ds(j*768, 768, 768)], sems.at[24 + slot])

            def wg_loop(name, lhs, rhs, dst, col0, t0, first, dx0):
                def body(i, _):
                    slot = (i + first) % 2
                    if first == 0:
                        @pl.when(i >= 2)
                        def _():
                            st_b(slot, dwin_h, 0).wait()
                    else:
                        st_b(slot, dwin_h, 0).wait()
                    t = jnp.minimum(t0 + i, 15)
                    for tile in range(1, 5):
                        goertzel(t, tile)
                    pgrad(t)
                    if dx0 is not None:
                        for j in range(3):
                            dx_tile(jnp.minimum(dx0 + 3*i + j, 15))
                    stg2[slot] = _pu(_dot(_bc(XG[lhs]), pk(rhs, i*768, 768), NT))
                    st_b(slot, dst, col0 + i).start()
                    return 0
                with jax.named_scope(name):
                    lax.fori_loop(0, 3, body, 0)
            wg_loop('win1', 0, ZY1, dwin_h, 0, 8, 0, 0)
            wg_loop('win2', 0, ZY2, dwin_h, 3, 11, 1, 9)
            cp(dxv, dxT_h.bitcast(u32), 21).start()
            wg_loop('wout', 1, YT, dwoutT_h, 0, 14, 2, None)
            finish()
            for s in range(2):
                st_a(s, slice(0, 128)).wait()
                st_b(s, dwin_h, 0).wait()
        pl.run_scoped(s2_scope, pltpu.VMEM((2, 128, L), u32), pltpu.VMEM((2, D//2, 768), u32))

        for c in final_copies():
            c.wait()
        cp(o1_v, ddsk_h, 20).wait()
        cp(dxv, dxT_h.bitcast(u32), 21).wait()

    pl.run_scoped(bwd_scope,
                  pltpu.VMEM((30, 16, 8, DP), f32), pltpu.VMEM((2, NG*8, DP), f32), pltpu.VMEM((4, 16, 8, DP), f32),
                  pltpu.VMEM((D//2, L), u32), pltpu.VMEM((DP, MP), f32), pltpu.VMEM((16, D, 128), f32),
                  pltpu.VMEM((8, DP), f32), pltpu.VMEM((7, 16, 8, DP), f32))


@jax.jit
def pallas_sequential_preLN__ssm_conv_s4__mixer_gmlp__prompt_kernel(
        A_u, A_A_re, A_A_im, A_B_re, A_B_im, A_C_re, A_C_im, A_log_dt, A_Dskip,
        B_x, B_w_in, B_w_sp, B_b_sp, B_w_out, grad_out):
    del B_x
    hbm = pl.BlockSpec(memory_space=pl.ANY)
    bf = lambda *s: jax.ShapeDtypeStruct(s, bf16)
    out_shape = (bf(D, L), bf(D, L)) + tuple(bf(D, N) for _ in range(6)) + (bf(D), bf(D), bf(D, F), bf(L, L), bf(L), bf(D, FH))
    V = pltpu.VMEM
    scratch = [
        V((2, D//2, L), u32),
        V((128, 128), u32), V((16, 128, 256), u32), V((64, 256), u32), V((19, 64, 128), u32),
        V((6, D, N), bf16), V((D,), bf16), V((D,), bf16), V((L,), bf16),
        V((6, 16, 8, DP), f32),
        V((1, DP), f32), V((D, 128), f32),
        V((16, D, 128), f32), V((16, D, 128), f32), V((16, L), f32),
        V((17, D, 128), u32), V((17, D, 128), u32),
        V((FH//2, L), u32), V((FH//2, L), u32), V((FH//2, L), u32), V((FH//2, L), u32), V((FH//2, L), u32),
        V((D,), bf16), V((D,), bf16), V((L,), bf16),
        pltpu.SemaphoreType.DMA((40,)),
    ]
    outs = pl.pallas_call(
        _kernel,
        out_shape=out_shape,
        in_specs=[hbm]*18,
        out_specs=[hbm]*14,
        scratch_shapes=scratch,
        compiler_params=pltpu.CompilerParams(vmem_limit_bytes=127*1024*1024),
    )(A_u.reshape(L, D).T, A_A_re, A_A_im, A_B_re, A_B_im, A_C_re, A_C_im, A_log_dt, A_Dskip,
      B_w_in, B_w_sp, B_b_sp, B_w_out.T, grad_out.reshape(L, D).T,
      jnp.asarray(C_F1), jnp.asarray(C_G), jnp.asarray(C_H), jnp.asarray(C_SEL))
    outT, dxT, dAre, dAim, dBre, dBim, dCre, dCim, dldt, ddsk, dwin, dwsp, dbsp, dwoutT = outs
    return (outT.T.reshape(1, L, D), dxT.T.reshape(1, L, D), dAre, dAim, dBre, dBim, dCre, dCim,
            dldt, ddsk, dwin, dwsp, dbsp, dwoutT.T)
```
